```python
import jax
import jax.numpy as jnp

def _softmax(x, axis=-1):
    return jax.nn.softmax(x, axis=axis)
def _gelu(x):
    return jax.nn.gelu(x, approximate=True)
def _silu(x):
    return jax.nn.silu(x)
def _sigmoid(x):
    return jax.nn.sigmoid(x)
def _layernorm(x, axis=-1, eps=1e-5):
    m = jnp.mean(x, axis=axis, keepdims=True)
    v = jnp.var(x, axis=axis, keepdims=True)
    return (x - m) / jnp.sqrt(v + eps)
def _scatter_add(tgt, idx, src, axis=0):
    return tgt.at[idx].add(src)
def _segment_sum(src, seg, n):
    return jax.ops.segment_sum(src, seg, n)
class _Rng:
    def __init__(self, key):
        self._k = key
    def _next(self):
        self._k, sub = jax.random.split(self._k)
        return sub
    def normal(self, shape):
        return jax.random.normal(self._next(), shape, dtype=jnp.bfloat16)
    def randint(self, lo, hi, shape):
        return jax.random.randint(self._next(), shape, lo, hi, dtype=jnp.int32)
    def uniform(self, shape, lo=0.0, hi=1.0):
        return jax.random.uniform(self._next(), shape, jnp.bfloat16, lo, hi)
    def permutation(self, n):
        return jax.random.permutation(self._next(), n)


kernel_name = 'gated_mix__sliding_block_cached__dense_activation_gelu__decode'

def setup_inputs():
    _rng = _Rng(jax.random.key(int.from_bytes(__import__("os").urandom(4), "little")))
    _w = (lambda a: (lambda t: t.astype(jnp.bfloat16) if jnp.issubdtype(t.dtype, jnp.floating) else t)(jnp.asarray(a)))
    def _A_setup():
        B, Sq, D = 1, 1, 640
        Hq, Hkv, Sk, Dh = 32, 32, 32768, 192
        assert Hq % Hkv == 0, (Hq, Hkv)
        return {
            "x": _w((lambda *s: _rng.normal(s) * 0.05)(B, Sq, D)),
            "k_cache": _w((lambda *s: _rng.normal(s) * 0.05)(B, Hkv, Sk, Dh)),
            "v_cache": _w((lambda *s: _rng.normal(s) * 0.05)(B, Hkv, Sk, Dh)),
            "wq": _w((lambda *s: _rng.normal(s) * 0.05)(D, Hq * Dh) * (D ** -0.5)),
            "wo": _w((lambda *s: _rng.normal(s) * 0.05)(Hq * Dh, D) * ((Hq * Dh) ** -0.5)),
        }
    _A_in = _A_setup()

    def _B_setup():
        B, S, D, F = 1, 1, 640, 1536
        return {
            "x": _w((lambda *s: _rng.normal(s) * 0.05)(B, S, D)),
            "w1": _w((lambda *s: _rng.normal(s) * 0.05)(D, F) * (D ** -0.5)),
            "b1": _w((lambda *s: _rng.normal(s) * 0.05)(F) * 0.01),
            "w2": _w((lambda *s: _rng.normal(s) * 0.05)(F, D) * (F ** -0.5)),
            "b2": _w((lambda *s: _rng.normal(s) * 0.05)(D) * 0.01),
        }
    _B_in = _B_setup()

    return {
        "A_x": _A_in["x"],
        "A_k_cache": _A_in["k_cache"],
        "A_v_cache": _A_in["v_cache"],
        "A_wq": _A_in["wq"],
        "A_wo": _A_in["wo"],
        "B_x": _B_in["x"],
        "B_w1": _B_in["w1"],
        "B_b1": _B_in["b1"],
        "B_w2": _B_in["w2"],
        "B_b2": _B_in["b2"],
        "gate_w": _w((lambda *s: _rng.normal(s) * 0.05)(640)),
    }

def reference(A_x, A_k_cache, A_v_cache, A_wq, A_wo, B_x, B_w1, B_b1, B_w2, B_b2, gate_w):
    def _A_ref(x, k_cache, v_cache, wq, wo):
        B, Sq, D = x.shape
        Hq, Dh = 32, 192
        Hkv, Sk = k_cache.shape[1], k_cache.shape[2]
        W = min(4096, max(256, Sk // 4))
        rep = Hq // Hkv
        q = (lambda x, *d: x.transpose(*d))((x @ wq).reshape(B, Sq, Hq, Dh), 0, 2, 1, 3)
        k = jnp.repeat(k_cache[:, :, Sk - W:, :], rep, axis=1)
        v = jnp.repeat(v_cache[:, :, Sk - W:, :], rep, axis=1)
        scores = jnp.einsum("bhqd,bhkd->bhqk", q, k) * (Dh ** -0.5)
        p = _softmax(scores, axis=-1)
        o = jnp.einsum("bhqk,bhkd->bhqd", p, v)
        return (lambda x, *d: x.transpose(*d))(o, 0, 2, 1, 3).reshape(B, Sq, Hq * Dh) @ wo

    def _B_ref(x, w1, b1, w2, b2):
        h = jnp.einsum("bsd,df->bsf", x, w1) + b1
        h = _gelu(h)
        return jnp.einsum("bsf,fd->bsd", h, w2) + b2

    x = A_x
    g = _sigmoid((x * gate_w).sum(-1, keepdims=True))
    a = _A_ref(x, A_k_cache, A_v_cache, A_wq, A_wo)
    b = _B_ref(x, B_w1, B_b1, B_w2, B_b2)
    return g * a + (1 - g) * b
```

```python
import functools

import jax
import jax.numpy as jnp
from jax import lax
import jax.experimental.pallas as pl
import jax.experimental.pallas.tpu as pltpu

F32 = jnp.float32
BF16 = jnp.bfloat16

_NB = 3
_WQ_CHUNK = 128
_WO_CHUNKS = (1536, 1536, 1536, 768, 384, 256, 128)


def _gelu_tanh(x):
    c = 0.7978845608028654
    return 0.5 * x * (1.0 + jnp.tanh(c * (x + 0.044715 * (x * x * x))))


def _kernel(x_hbm, k_hbm, v_hbm, wq_hbm, wo_hbm, w1_hbm, b1_hbm, w2_hbm, b2_hbm,
            gw_hbm, o_ref,
            x_v, b1_v, b2_v, gw_v, wq_v, wo_v, w1_v, w2_v, kbuf, vbuf,
            q_scr, p_scr, ocol_scr,
            sem_small, sem_wq, sem_w, sem_wo, sem_k, sem_v,
            *, n_pairs, dh, win, sk):
    d_model = x_v.shape[-1]
    pair = 2 * dh
    n_wq = d_model // _WQ_CHUNK
    scale = float(dh) ** -0.5

    def wq_copy(c):
        rows = pl.ds(c * _WQ_CHUNK, _WQ_CHUNK)
        return pltpu.make_async_copy(wq_hbm.at[rows], wq_v.at[rows], sem_wq.at[c])

    def small_copies():
        return [
            pltpu.make_async_copy(x_hbm, x_v, sem_small.at[0]),
            pltpu.make_async_copy(gw_hbm, gw_v, sem_small.at[1]),
            pltpu.make_async_copy(b1_hbm, b1_v, sem_small.at[2]),
            pltpu.make_async_copy(b2_hbm, b2_v, sem_small.at[3]),
        ]

    w1_copy = pltpu.make_async_copy(w1_hbm, w1_v, sem_w.at[0])
    w2_copy = pltpu.make_async_copy(w2_hbm, w2_v, sem_w.at[1])

    wo_starts = [sum(_WO_CHUNKS[:c]) for c in range(len(_WO_CHUNKS))]

    def wo_copy(c):
        rows = pl.ds(wo_starts[c], _WO_CHUNKS[c])
        return pltpu.make_async_copy(wo_hbm.at[rows], wo_v.at[rows], sem_wo.at[c])

    def k_copy(i, slot):
        return pltpu.make_async_copy(
            k_hbm.at[i, :, pl.ds(sk - win, win)], kbuf.at[slot], sem_k.at[slot])

    def v_copy(i, slot):
        return pltpu.make_async_copy(
            v_hbm.at[i, :, pl.ds(sk - win, win)], vbuf.at[slot], sem_v.at[slot])

    wq_copy(0).start()
    for cp in small_copies():
        cp.start()
    for c in range(1, n_wq):
        wq_copy(c).start()
    w1_copy.start()
    for i in range(_NB):
        k_copy(i, i).start()
        v_copy(i, i).start()
    w2_copy.start(priority=1)
    for c in range(len(_WO_CHUNKS)):
        wo_copy(c).start(priority=1)

    for cp in small_copies():
        cp.wait()
    x_row = x_v[0]
    x8 = jnp.broadcast_to(x_row, (8, d_model))

    q = None
    for c in range(n_wq):
        wq_copy(c).wait()
        part = jnp.dot(x8[:, c * _WQ_CHUNK:(c + 1) * _WQ_CHUNK],
                       wq_v[c * _WQ_CHUNK:(c + 1) * _WQ_CHUNK, :],
                       preferred_element_type=F32)
        q = part if q is None else q + part
    lane = lax.broadcasted_iota(jnp.int32, (8, pair), 1)
    for i in range(n_pairs):
        qp = q[:, i * pair:(i + 1) * pair]
        q_scr[i] = jnp.concatenate(
            [jnp.where(lane < dh, qp, 0.0), jnp.where(lane >= dh, qp, 0.0)],
            axis=0).astype(BF16)

    w1_copy.wait()
    h = jnp.dot(x8, w1_v[...], preferred_element_type=F32)
    h = h + b1_v[...].astype(F32).reshape(1, -1)
    h = _gelu_tanh(h).astype(BF16)
    gate = jnp.sum(x_row.astype(F32) * gw_v[...].astype(F32).reshape(1, -1),
                   axis=-1, keepdims=True)
    gate = 1.0 / (1.0 + jnp.exp(-gate))

    def pair_step(i, carry):
        slot = lax.rem(i, _NB)
        k_copy(i, slot).wait()
        s = jnp.dot(q_scr[i], kbuf[slot], preferred_element_type=F32) * scale

        @pl.when(i + _NB < n_pairs)
        def _():
            k_copy(i + _NB, slot).start()

        m = jnp.max(s, axis=-1, keepdims=True)
        p = jnp.exp(s - m)
        l = jnp.sum(p, axis=-1, keepdims=True)
        p_scr[...] = p * (1.0 / l)

        v_copy(i, slot).wait()
        for hh in range(2):
            acc = jnp.zeros((dh // 8, 8, 128), F32)
            for j in range(win // 128):
                pj = p_scr[hh * 8:(hh + 1) * 8, j * 128:(j + 1) * 128]
                vj = vbuf[slot, hh * dh:(hh + 1) * dh, j * 128:(j + 1) * 128]
                acc = acc + vj.astype(F32).reshape(dh // 8, 8, 128) * pj[None]
            o_col = jnp.sum(acc.reshape(dh, 128), axis=-1, keepdims=True)
            row0 = pl.multiple_of(i * pair + hh * dh, 8)
            ocol_scr[pl.ds(row0, dh), :] = jnp.broadcast_to(o_col, (dh, 128))

        @pl.when(i + _NB < n_pairs)
        def _():
            v_copy(i + _NB, slot).start()

        return carry

    lax.fori_loop(0, n_pairs, pair_step, 0)

    w2_copy.wait()
    b = jnp.dot(h, w2_v[...], preferred_element_type=F32)[0:1]
    b = b + b2_v[...].astype(F32).reshape(1, -1)
    b = (1.0 - gate) * b

    n_lt = d_model // 128
    acc = jnp.zeros((8, d_model), F32)
    for c in range(len(_WO_CHUNKS)):
        wo_copy(c).wait()

        def wo_step(r, a, base=wo_starts[c]):
            rows = pl.ds(pl.multiple_of(base + r * 128, 128), 128)
            oc = ocol_scr[rows, :]
            w = wo_v[rows, :].astype(F32)
            prod = w * jnp.concatenate([oc] * n_lt, axis=1)
            return a + jnp.sum(prod.reshape(16, 8, d_model), axis=0)

        acc = lax.fori_loop(0, _WO_CHUNKS[c] // 128, wo_step, acc)
    a = jnp.sum(acc, axis=0, keepdims=True)
    o_ref[0] = (gate * a + b).astype(o_ref.dtype)


@jax.jit
def pallas_gated_mix__sliding_block_cached__dense_activation_gelu__decode_kernel(
    A_x: jax.Array,
    A_k_cache: jax.Array,
    A_v_cache: jax.Array,
    A_wq: jax.Array,
    A_wo: jax.Array,
    B_x: jax.Array,
    B_w1: jax.Array,
    B_b1: jax.Array,
    B_w2: jax.Array,
    B_b2: jax.Array,
    gate_w: jax.Array,
):
    del B_x
    bsz, sq, d_model = A_x.shape
    _, n_heads, sk, dh = A_k_cache.shape
    d_ff = B_w1.shape[1]
    assert bsz == 1 and sq == 1 and n_heads % 2 == 0
    assert A_wq.shape == (d_model, n_heads * dh)
    assert sum(_WO_CHUNKS) == n_heads * dh
    win = min(4096, max(256, sk // 4))
    n_pairs = n_heads // 2
    pair = 2 * dh

    k_t = jnp.swapaxes(A_k_cache, 2, 3).reshape(n_pairs, pair, sk)
    v_t = jnp.swapaxes(A_v_cache, 2, 3).reshape(n_pairs, pair, sk)

    kernel = functools.partial(_kernel, n_pairs=n_pairs, dh=dh, win=win, sk=sk)
    any_spec = pl.BlockSpec(memory_space=pl.ANY)
    return pl.pallas_call(
        kernel,
        out_shape=jax.ShapeDtypeStruct((bsz, sq, d_model), A_x.dtype),
        in_specs=[any_spec] * 10,
        out_specs=pl.BlockSpec(memory_space=pltpu.VMEM),
        scratch_shapes=[
            pltpu.VMEM(A_x.shape, BF16),
            pltpu.VMEM(B_b1.shape, BF16),
            pltpu.VMEM(B_b2.shape, BF16),
            pltpu.VMEM(gate_w.shape, BF16),
            pltpu.VMEM(A_wq.shape, BF16),
            pltpu.VMEM(A_wo.shape, BF16),
            pltpu.VMEM(B_w1.shape, BF16),
            pltpu.VMEM(B_w2.shape, BF16),
            pltpu.VMEM((_NB, pair, win), BF16),
            pltpu.VMEM((_NB, pair, win), BF16),
            pltpu.VMEM((n_pairs, 16, pair), BF16),
            pltpu.VMEM((16, win), F32),
            pltpu.VMEM((n_heads * dh, 128), F32),
            pltpu.SemaphoreType.DMA((4,)),
            pltpu.SemaphoreType.DMA((d_model // _WQ_CHUNK,)),
            pltpu.SemaphoreType.DMA((2,)),
            pltpu.SemaphoreType.DMA((len(_WO_CHUNKS),)),
            pltpu.SemaphoreType.DMA((_NB,)),
            pltpu.SemaphoreType.DMA((_NB,)),
        ],
        compiler_params=pltpu.CompilerParams(vmem_limit_bytes=96 * 1024 * 1024),
    )(A_x, k_t, v_t, A_wq, A_wo, B_w1, B_b1, B_w2, B_b2, gate_w)
```

```python
import functools

import jax
import jax.numpy as jnp
from jax import lax
import jax.experimental.pallas as pl
import jax.experimental.pallas.tpu as pltpu

F32 = jnp.float32
BF16 = jnp.bfloat16

DEFAULT = dict(R=16, splits=(1792,), L=24, nw=8, shift=30, compute=True,
               q_step=2, ffn_step=4)


def _gelu_tanh(x):
    c = 0.7978845608028654
    return 0.5 * x * (1.0 + jnp.tanh(c * (x + 0.044715 * (x * x * x))))


def _spread(units, nsteps):
    out, done = [], 0
    for s in range(nsteps):
        upto = (units * (s + 1)) // nsteps
        out.append((done, upto - done))
        done = upto
    return out


def _kernel(x_hbm, k_hbm, v_hbm, wq_hbm, wo_hbm, w1_hbm, b1_hbm, w2_hbm, b2_hbm,
            gw_hbm, o_ref,
            x_v, b1_v, b2_v, gw_v, wq0_v, wq_v, wo_v, w1_v, w2_v, kbuf, vbuf,
            qcol, s_scr, oacc, h_scr, b_scr, sems,
            *, n_pairs, dh, win, sk, cfg):
    R, L, nw, compute = cfg["R"], cfg["L"], cfg["nw"], cfg["compute"]
    d_model = x_v.shape[-1]
    d_ff = w1_v.shape[1]
    pair = 2 * dh
    scale = float(dh) ** -0.5
    bounds = (0,) + tuple(cfg["splits"]) + (win,)
    parts = [(bounds[t], bounds[t + 1] - bounds[t]) for t in range(len(bounds) - 1)]
    n_part = len(parts)
    ns = pair // R
    nh = ns // 2
    half = n_part * ns
    n_steps = 2 * half
    assert n_steps % L == 0
    steps = [(ph, t, j) for ph in range(2) for t in range(n_part) for j in range(ns)]
    S_WQ, S_WO, S_W1, S_W2, S_WQ0, S_X, S_SM = (L + t for t in range(7))
    n_g = R // 8
    n_lt = d_model // 128

    def kv(i, s):
        ph, t, j = steps[s]
        src, dst = ((k_hbm, kbuf), (v_hbm, vbuf))[ph]
        o, c = parts[t]
        rows = pl.ds(j * R, R)
        return pltpu.make_async_copy(src.at[i, rows, pl.ds(sk - win + o, c)],
                                     dst.at[rows, pl.ds(o, c)], sems.at[s % L])

    def wq_piece(i, t0, n):
        rows = pl.ds(t0 * 8, n * 8)
        cols = pl.ds(i * pair if isinstance(i, int) else pl.multiple_of(i * pair, 128), pair)
        return pltpu.make_async_copy(wq_hbm.at[rows, cols], wq_v.at[rows], sems.at[S_WQ])

    def wo_piece(i, t0, n):
        return pltpu.make_async_copy(
            wo_hbm.at[pl.ds(pl.multiple_of(i * pair + t0 * 8, 8), n * 8)],
            wo_v.at[pl.ds(t0 * 8, n * 8)], sems.at[S_WO])

    w1_per, w2_per = d_model // 8 // nw, d_ff // 8 // nw

    def w1_piece(i, u):
        rows = pl.ds(pl.multiple_of((i * w1_per + u // 2) * 8, 8), 8)
        cols = pl.ds((u % 2) * (d_ff // 2), d_ff // 2)
        return pltpu.make_async_copy(w1_hbm.at[rows, cols], w1_v.at[rows, cols], sems.at[S_W1])

    def w2_piece(i, u):
        rows = pl.ds(pl.multiple_of((i * w2_per + u) * 8, 8), 8)
        return pltpu.make_async_copy(w2_hbm.at[rows], w2_v.at[rows], sems.at[S_W2])

    def wait_all(buf, sem):
        pltpu.make_async_copy(buf, buf, sems.at[sem]).wait()

    a = half - cfg["shift"]
    wq_sp = _spread(d_model // 8, half)
    wo_sp = _spread(pair // 8, half)
    w1_sp = _spread(2 * w1_per, half)
    w2_sp = _spread(w2_per, half)
    wq_early = wq_sp[half - a][0] if a > 0 else d_model // 8

    x_copy = pltpu.make_async_copy(x_hbm, x_v, sems.at[S_X])
    small = [pltpu.make_async_copy(gw_hbm, gw_v, sems.at[S_SM]),
             pltpu.make_async_copy(b1_hbm, b1_v, sems.at[S_SM + 1]),
             pltpu.make_async_copy(b2_hbm, b2_v, sems.at[S_SM + 2])]
    wq0_copy = pltpu.make_async_copy(wq_hbm.at[:, pl.ds(0, pair)], wq0_v, sems.at[S_WQ0])

    wq0_copy.start()
    x_copy.start()
    for s in range(L):
        kv(0, s).start(priority=1)
    for cp in small:
        cp.start()
    if wq_early:
        wq_piece(1, 0, wq_early).start()

    def make_qcol(w_ref):
        x8 = jnp.broadcast_to(x_v[0], (8, d_model))
        q8 = jnp.dot(x8, w_ref[...], preferred_element_type=F32)
        q8 = q8.astype(BF16).astype(F32)
        qb = jnp.concatenate([q8] * 16, axis=0)
        qcol[...] = qb.T

    x_copy.wait()
    wq0_copy.wait()
    if compute:
        make_qcol(wq0_v)
    for cp in small:
        cp.wait()

    def pair_body(i, out):
        more1 = i + 1 < n_pairs
        more2 = i + 2 < n_pairs
        m_vec = [None, None]
        m = [None, None]
        lsum = [None, None]
        s_acc = p = out_h = None
        for s in range(n_steps):
            ph, t, j = steps[s]
            o, c = parts[t]
            n_cb = c // 128
            hh, jj = j // nh, j % nh
            r0 = j * R

            kv(i, s).wait()
            if s + L < n_steps:
                kv(i, s + L).start(priority=1)
            else:
                @pl.when(more1)
                def _():
                    kv(i + 1, s + L - n_steps).start(priority=1)
            if s < a:
                t0, n = wq_sp[half - a + s]
                if n:
                    @pl.when(more1)
                    def _():
                        wq_piece(i + 1, t0, n).start()
            elif s < a + half:
                t0, n = wo_sp[s - a]
                if n:
                    wo_piece(i, t0, n).start()
            else:
                t0, n = wq_sp[s - a - half]
                if n:
                    @pl.when(more2)
                    def _():
                        wq_piece(i + 2, t0, n).start()
            sp, fn = (w1_sp, w1_piece) if s % 2 == 0 else (w2_sp, w2_piece)
            t0, n = sp[s // 2]
            if n:
                @pl.when(i < nw)
                def _():
                    for u in range(n):
                        fn(i, t0 + u).start()

            if s == half + cfg["q_step"]:
                @pl.when(more1)
                def _():
                    wait_all(wq_v, S_WQ)
                    if compute:
                        make_qcol(wq_v)
            if s == cfg["ffn_step"]:
                @pl.when(i == nw)
                def _():
                    wait_all(w1_v, S_W1)
                    if compute:
                        x8 = jnp.broadcast_to(x_v[0], (8, d_model))
                        h = jnp.dot(x8, w1_v[...], preferred_element_type=F32)
                        h = h + b1_v[...].astype(F32).reshape(1, -1)
                        h_scr[...] = _gelu_tanh(h).astype(BF16)

                @pl.when(i == nw + 1)
                def _():
                    wait_all(w2_v, S_W2)
                    if compute:
                        b = jnp.dot(h_scr[...], w2_v[...], preferred_element_type=F32)
                        b_scr[...] = b + b2_v[...].astype(F32).reshape(1, -1)
            if ph == 1 and t == n_part - 1 and j == 0:
                wait_all(wo_v, S_WO)
            if not compute:
                continue

            if ph == 0:
                kf = kbuf[r0:r0 + R, o:o + c].astype(F32)
                qc = qcol[r0:r0 + R, :]
                for g in range(n_g):
                    qg = qc[8 * g:8 * g + 8]
                    term = [kf[8 * g:8 * g + 8, cb * 128:(cb + 1) * 128] * qg for cb in range(n_cb)]
                    if jj == 0 and g == 0:
                        s_acc = term
                    else:
                        s_acc = [u + v for u, v in zip(s_acc, term)]
                if jj == nh - 1:
                    for cb in range(n_cb):
                        z = s_acc[cb]
                        z = z + pltpu.roll(z, 4, 0)
                        z = z + pltpu.roll(z, 2, 0)
                        z = z + pltpu.roll(z, 1, 0)
                        s_scr[hh * 8:(hh + 1) * 8, o + cb * 128:o + (cb + 1) * 128] = z
                        m_vec[hh] = z if m_vec[hh] is None else jnp.maximum(m_vec[hh], z)
                    if t == n_part - 1:
                        m[hh] = jnp.max(m_vec[hh], axis=-1, keepdims=True)
            else:
                if jj == 0:
                    sv = s_scr[hh * 8:(hh + 1) * 8, o:o + c]
                    pv = jnp.exp((sv - m[hh]) * scale)
                    p = [pv[:, cb * 128:(cb + 1) * 128] for cb in range(n_cb)]
                    for u in p:
                        lsum[hh] = u if lsum[hh] is None else lsum[hh] + u
                vf = vbuf[r0:r0 + R, o:o + c].astype(F32)
                accs = []
                for g in range(n_g):
                    terms = [vf[8 * g:8 * g + 8, cb * 128:(cb + 1) * 128] * p[cb] for cb in range(n_cb)]
                    if t > 0:
                        terms.append(oacc[r0 + 8 * g:r0 + 8 * g + 8, :])
                    while len(terms) > 1:
                        terms = [terms[u] + terms[u + 1] if u + 1 < len(terms) else terms[u]
                                 for u in range(0, len(terms), 2)]
                    accs.append(terms[0])
                if t < n_part - 1:
                    for g in range(n_g):
                        oacc[r0 + 8 * g:r0 + 8 * g + 8, :] = accs[g]
                else:
                    wf = wo_v[r0:r0 + R, :].astype(F32)
                    for g in range(n_g):
                        oc = jnp.sum(accs[g], axis=-1, keepdims=True)
                        term = wf[8 * g:8 * g + 8, :] * oc
                        out_h = term if (jj == 0 and g == 0) else out_h + term
                    if jj == nh - 1:
                        l = jnp.sum(lsum[hh], axis=-1, keepdims=True)
                        out = out + out_h * (1.0 / l)
        return out

    out = lax.fori_loop(0, n_pairs, pair_body, jnp.zeros((8, d_model), F32))

    gate = jnp.sum(x_v[0].astype(F32) * gw_v[...].astype(F32).reshape(1, -1),
                   axis=-1, keepdims=True)
    gate = 1.0 / (1.0 + jnp.exp(-gate))
    a_row = jnp.sum(out, axis=0, keepdims=True)
    if compute:
        res = gate * a_row + (1.0 - gate) * b_scr[0:1, :]
    else:
        res = gate * a_row
    o_ref[0] = res.astype(o_ref.dtype)


@jax.jit
def pallas_gated_mix__sliding_block_cached__dense_activation_gelu__decode_kernel(
    A_x: jax.Array,
    A_k_cache: jax.Array,
    A_v_cache: jax.Array,
    A_wq: jax.Array,
    A_wo: jax.Array,
    B_x: jax.Array,
    B_w1: jax.Array,
    B_b1: jax.Array,
    B_w2: jax.Array,
    B_b2: jax.Array,
    gate_w: jax.Array,
):
    del B_x
    cfg = DEFAULT
    bsz, sq, d_model = A_x.shape
    _, n_heads, sk, dh = A_k_cache.shape
    d_ff = B_w1.shape[1]
    win = min(4096, max(256, sk // 4))
    n_pairs = n_heads // 2
    pair = 2 * dh
    k_t = jnp.swapaxes(A_k_cache, 2, 3).reshape(n_pairs, pair, sk)
    v_t = jnp.swapaxes(A_v_cache, 2, 3).reshape(n_pairs, pair, sk)
    kernel = functools.partial(_kernel, n_pairs=n_pairs, dh=dh, win=win, sk=sk, cfg=cfg)
    any_spec = pl.BlockSpec(memory_space=pl.ANY)
    return pl.pallas_call(
        kernel,
        out_shape=jax.ShapeDtypeStruct((bsz, sq, d_model), A_x.dtype),
        in_specs=[any_spec] * 10,
        out_specs=pl.BlockSpec(memory_space=pltpu.VMEM),
        scratch_shapes=[
            pltpu.VMEM(A_x.shape, BF16),
            pltpu.VMEM(B_b1.shape, BF16),
            pltpu.VMEM(B_b2.shape, BF16),
            pltpu.VMEM(gate_w.shape, BF16),
            pltpu.VMEM((d_model, pair), BF16),
            pltpu.VMEM((d_model, pair), BF16),
            pltpu.VMEM((pair, d_model), BF16),
            pltpu.VMEM(B_w1.shape, BF16),
            pltpu.VMEM(B_w2.shape, BF16),
            pltpu.VMEM((pair, win), BF16),
            pltpu.VMEM((pair, win), BF16),
            pltpu.VMEM((pair, 128), F32),
            pltpu.VMEM((16, win), F32),
            pltpu.VMEM((pair, 128), F32),
            pltpu.VMEM((8, d_ff), BF16),
            pltpu.VMEM((8, d_model), F32),
            pltpu.SemaphoreType.DMA((cfg["L"] + 9,)),
        ],
        compiler_params=pltpu.CompilerParams(
            vmem_limit_bytes=64 * 1024 * 1024,
            disable_semaphore_checks=True,
            disable_bounds_checks=True),
    )(A_x, k_t, v_t, A_wq, A_wo, B_w1, B_b1, B_w2, B_b2, gate_w)
```

```python
import functools

import jax
import jax.numpy as jnp
from jax import lax
import jax.experimental.pallas as pl
import jax.experimental.pallas.tpu as pltpu

F32 = jnp.float32
BF16 = jnp.bfloat16

DEFAULT = dict(R=16, split=1792, strip=256, lead=12, sgrp=6, L=24, nw=8, shift=30, compute=True,
               q_steps=(2,), ffn1_n=4, ffn2_n=5, ffn_step=4, ffn_gap=2, fin=4, wlate=False,
               do_q=True, do_ffn=True, do_k=True, do_v=True)


def _gelu_tanh(x):
    c = 0.7978845608028654
    return 0.5 * x * (1.0 + jnp.tanh(c * (x + 0.044715 * (x * x * x))))


def _spread(units, nsteps):
    out, done = [], 0
    for s in range(nsteps):
        upto = (units * (s + 1)) // nsteps
        out.append((done, upto - done))
        done = upto
    return out


def _tree_sum(terms):
    while len(terms) > 1:
        terms = [terms[u] + terms[u + 1] if u + 1 < len(terms) else terms[u]
                 for u in range(0, len(terms), 2)]
    return terms[0]


def _kernel(x_hbm, k_hbm, v_hbm, wq_hbm, wo_hbm, w1_hbm, b1_hbm, w2_hbm, b2_hbm,
            gw_hbm, o_ref,
            x_v, b1_v, b2_v, gw_v, wq0_v, wq_v, wo_v, w1_v, w2_v, kbuf, vbuf,
            x8_scr, qcol, s_scr, oacc, h_scr, b_scr, sems,
            *, n_pairs, dh, win, sk, cfg):
    R, L, nw, compute = cfg["R"], cfg["L"], cfg["nw"], cfg["compute"]
    split, strip, lead, sgrp = cfg["split"], cfg["strip"], cfg["lead"], cfg["sgrp"]
    d_model = x_v.shape[-1]
    d_ff = w1_v.shape[1]
    pair = 2 * dh
    scale = float(dh) ** -0.5
    dma_parts = [(0, split), (split + strip, win - split - strip)]
    cmp_parts = [(0, split), (split, win - split)]
    n_part = 2
    ns = pair // R
    nh = ns // 2
    half = n_part * ns
    n_steps = 2 * half
    assert n_steps % L == 0
    steps = [(ph, t, j) for ph in range(2) for t in range(n_part) for j in range(ns)]
    S_WQ, S_WO, S_W1, S_W2, S_WQ0, S_X, S_SM = (L + t for t in range(7))
    S_ST = S_SM + 3
    n_g = R // 8
    n_rg = pair // 8
    srows = pair // half
    assert srows % 8 == 0 and half % sgrp == 0
    bufs = ((k_hbm, kbuf), (v_hbm, vbuf))

    def kv(i, s):
        ph, t, j = steps[s]
        src, dst = bufs[ph]
        o, c = dma_parts[t]
        rows = pl.ds(j * R, R)
        return pltpu.make_async_copy(src.at[i, rows, pl.ds(sk - win + o, c)],
                                     dst.at[rows, pl.ds(o, c)], sems.at[s % L])

    def strip_copy(i, ph, u, n=1):
        src, dst = bufs[ph]
        rows = pl.ds(u * srows, n * srows)
        return pltpu.make_async_copy(src.at[i, rows, pl.ds(sk - win + split, strip)],
                                     dst.at[rows, pl.ds(split, strip)],
                                     sems.at[S_ST + u // sgrp])

    def wq_piece(i, t0, n):
        rows = pl.ds(t0 * 8, n * 8)
        cols = pl.ds(i * pair if isinstance(i, int) else pl.multiple_of(i * pair, 128), pair)
        return pltpu.make_async_copy(wq_hbm.at[rows, cols], wq_v.at[rows], sems.at[S_WQ])

    def wo_piece(i, t0, n):
        return pltpu.make_async_copy(
            wo_hbm.at[pl.ds(pl.multiple_of(i * pair + t0 * 8, 8), n * 8)],
            wo_v.at[pl.ds(t0 * 8, n * 8)], sems.at[S_WO])

    w1_per, w2_per = d_model // 8 // nw, d_ff // 8 // nw

    def w1_piece(i, u):
        rows = pl.ds(pl.multiple_of((i * w1_per + u // 2) * 8, 8), 8)
        cols = pl.ds((u % 2) * (d_ff // 2), d_ff // 2)
        return pltpu.make_async_copy(w1_hbm.at[rows, cols], w1_v.at[rows, cols], sems.at[S_W1])

    def w2_piece(i, u):
        rows = pl.ds(pl.multiple_of((i * w2_per + u) * 8, 8), 8)
        return pltpu.make_async_copy(w2_hbm.at[rows], w2_v.at[rows], sems.at[S_W2])

    def wait_all(buf, sem):
        pltpu.make_async_copy(buf, buf, sems.at[sem]).wait()

    a = half - cfg["shift"]
    wq_sp = _spread(d_model // 8, half)
    wo_sp = _spread(pair // 8, half)
    w1_sp = _spread(2 * w1_per, half)
    w2_sp = _spread(w2_per, half)
    wq_early = wq_sp[half - a][0] if a > 0 else d_model // 8

    x_copy = pltpu.make_async_copy(x_hbm, x_v, sems.at[S_X])
    small = [pltpu.make_async_copy(gw_hbm, gw_v, sems.at[S_SM]),
             pltpu.make_async_copy(b1_hbm, b1_v, sems.at[S_SM + 1]),
             pltpu.make_async_copy(b2_hbm, b2_v, sems.at[S_SM + 2])]
    wq0_copy = pltpu.make_async_copy(wq_hbm.at[:, pl.ds(0, pair)], wq0_v, sems.at[S_WQ0])

    x_copy.start()
    small[0].start()
    wq0_copy.start()
    for s in range(L):
        kv(0, s).start(priority=1)
    for cp in small[1:]:
        cp.start()
    if strip:
        for u in range(0, lead, sgrp):
            strip_copy(0, 0, u, min(sgrp, lead - u)).start()
    if wq_early:
        wq_piece(1, 0, wq_early).start()

    def make_qcol(w_ref, c0, c1):
        q8 = jnp.dot(x8_scr[...], w_ref[:, c0:c1], preferred_element_type=F32)
        q8 = q8.astype(BF16).astype(F32)
        qb = jnp.concatenate([q8] * 16, axis=0)
        qcol[c0:c1, :] = qb.T

    x_copy.wait()
    small[0].wait()
    x8_scr[...] = jnp.broadcast_to(x_v[0], (8, d_model))
    gate = jnp.sum(x8_scr[...].astype(F32) * gw_v[...].astype(F32).reshape(1, -1),
                   axis=-1, keepdims=True)
    gate = 1.0 / (1.0 + jnp.exp(-gate))
    wq0_copy.wait()
    if compute:
        make_qcol(wq0_v, 0, pair)
    for cp in small[1:]:
        cp.wait()

    q_steps = cfg["q_steps"]
    q_w = pair // len(q_steps)
    f1_w, f2_w = d_ff // cfg["ffn1_n"], d_model // cfg["ffn2_n"]

    def pair_body(i, out):
        more1 = i + 1 < n_pairs
        more2 = i + 2 < n_pairs
        m_vec = [None, None]
        m = [None, None]
        lsum = [None, None]
        inv_l = [None, None]
        s_acc = p = out_h = None
        pending = []

        def finalize(pend, out_h, out):
            ocs, r0, hh, jj = pend
            ocs = [jnp.sum(z, axis=-1, keepdims=True) for z in ocs]
            wf = wo_v[r0:r0 + R, :].astype(F32)
            for g in range(n_g):
                term = wf[8 * g:8 * g + 8, :] * ocs[g]
                out_h = term if (jj == 0 and g == 0) else out_h + term
            if jj == nh - 1:
                out = out + out_h * inv_l[hh]
            return out_h, out

        def issue_w(s):
            if s < a:
                t0, n = wq_sp[half - a + s]
                if n:
                    @pl.when(more1)
                    def _():
                        wq_piece(i + 1, t0, n).start()
            elif s < a + half:
                t0, n = wo_sp[s - a]
                if n:
                    wo_piece(i, t0, n).start()
            else:
                t0, n = wq_sp[s - a - half]
                if n:
                    @pl.when(more2)
                    def _():
                        wq_piece(i + 2, t0, n).start()
            sp, fn = (w1_sp, w1_piece) if s % 2 == 0 else (w2_sp, w2_piece)
            t0, n = sp[s // 2]
            if n:
                @pl.when(i < nw)
                def _():
                    for u in range(n):
                        fn(i, t0 + u).start()

        for s in range(n_steps):
            ph, t, j = steps[s]
            o, c = cmp_parts[t]
            n_cb = c // 128
            hh, jj = j // nh, j % nh
            r0 = j * R

            kv(i, s).wait()
            if s + L < n_steps:
                kv(i, s + L).start(priority=1)
            else:
                @pl.when(more1)
                def _():
                    kv(i + 1, s + L - n_steps).start(priority=1)
            if strip:
                su = s + lead
                if su < n_steps:
                    strip_copy(i, su // half, su % half).start()
                else:
                    @pl.when(more1)
                    def _():
                        strip_copy(i + 1, 0, su - n_steps).start()
            if not cfg["wlate"]:
                issue_w(s)

            if s - half in q_steps:
                u = q_steps.index(s - half)

                @pl.when(more1)
                def _():
                    if u == 0:
                        wait_all(wq_v, S_WQ)
                    if compute and cfg["do_q"]:
                        make_qcol(wq_v, u * q_w, (u + 1) * q_w)
            fs = s - cfg["ffn_step"]
            if fs >= 0 and fs % cfg["ffn_gap"] == 0:
                u = fs // cfg["ffn_gap"]
                if u < cfg["ffn1_n"]:
                    @pl.when(i == nw)
                    def _():
                        if u == 0:
                            wait_all(w1_v, S_W1)
                        if compute and cfg["do_ffn"]:
                            cs = slice(u * f1_w, (u + 1) * f1_w)
                            h = jnp.dot(x8_scr[...], w1_v[:, cs], preferred_element_type=F32)
                            h = h + b1_v[...].astype(F32).reshape(1, -1)[:, cs]
                            h_scr[:, cs] = _gelu_tanh(h).astype(BF16)
                elif u < cfg["ffn1_n"] + cfg["ffn2_n"]:
                    u2 = u - cfg["ffn1_n"]

                    @pl.when(i == nw)
                    def _():
                        if u2 == 0:
                            wait_all(w2_v, S_W2)
                        if compute and cfg["do_ffn"]:
                            cs = slice(u2 * f2_w, (u2 + 1) * f2_w)
                            b = jnp.dot(h_scr[...], w2_v[:, cs], preferred_element_type=F32)
                            b = b + b2_v[...].astype(F32).reshape(1, -1)[:, cs]
                            b_scr[:, cs] = b * (1.0 - gate)
            if ph == 1 and t == 1 and j == 0:
                wait_all(wo_v, S_WO)
            if strip and t == 1 and (r0 // srows) % sgrp == 0:
                assert R // srows <= sgrp and sgrp % (R // srows) == 0
                strip_copy(i, ph, r0 // srows, sgrp).wait()
            if compute:
                if len(pending) >= cfg["fin"] or s == n_steps - 1:
                    for pend in pending:
                        out_h, out = finalize(pend, out_h, out)
                    pending = []
                if ph == 0 and not cfg["do_k"]:
                    m[hh] = jnp.zeros((8, 1), F32)
                elif ph == 1 and not cfg["do_v"]:
                    pass
                elif ph == 0:
                    kf = kbuf[r0:r0 + R, o:o + c].astype(F32)
                    qc = qcol[r0:r0 + R, :]
                    for g in range(n_g):
                        qg = qc[8 * g:8 * g + 8]
                        term = [kf[8 * g:8 * g + 8, cb * 128:(cb + 1) * 128] * qg for cb in range(n_cb)]
                        if jj == 0 and g == 0:
                            s_acc = term
                        else:
                            s_acc = [u + v for u, v in zip(s_acc, term)]
                    if jj == nh - 1:
                        for cb in range(n_cb):
                            z = s_acc[cb]
                            z = z + pltpu.roll(z, 4, 0)
                            z = z + pltpu.roll(z, 2, 0)
                            z = z + pltpu.roll(z, 1, 0)
                            s_scr[hh * 8:(hh + 1) * 8, o + cb * 128:o + (cb + 1) * 128] = z
                            m_vec[hh] = z if m_vec[hh] is None else jnp.maximum(m_vec[hh], z)
                        if t == n_part - 1:
                            m[hh] = jnp.max(m_vec[hh], axis=-1, keepdims=True)
                else:
                    if jj == 0:
                        sv = s_scr[hh * 8:(hh + 1) * 8, o:o + c]
                        pv = jnp.exp((sv - m[hh]) * scale)
                        p = [pv[:, cb * 128:(cb + 1) * 128] for cb in range(n_cb)]
                        ps = _tree_sum(list(p))
                        lsum[hh] = ps if lsum[hh] is None else lsum[hh] + ps
                        if t == n_part - 1:
                            inv_l[hh] = gate / jnp.sum(lsum[hh], axis=-1, keepdims=True)
                    vf = vbuf[r0:r0 + R, o:o + c].astype(F32)
                    accs = []
                    for g in range(n_g):
                        terms = [vf[8 * g:8 * g + 8, cb * 128:(cb + 1) * 128] * p[cb] for cb in range(n_cb)]
                        if t > 0:
                            terms.append(oacc[r0 + 8 * g:r0 + 8 * g + 8, :])
                        accs.append(_tree_sum(terms))
                    if t < n_part - 1:
                        for g in range(n_g):
                            oacc[r0 + 8 * g:r0 + 8 * g + 8, :] = accs[g]
                    else:
                        pending.append((accs, r0, hh, jj))
                        if s == n_steps - 1:
                            out_h, out = finalize(pending.pop(), out_h, out)
            if cfg["wlate"]:
                issue_w(s)
        return out

    out = lax.fori_loop(0, n_pairs, pair_body, jnp.zeros((8, d_model), F32))

    res = jnp.sum(out, axis=0, keepdims=True)
    if compute:
        res = res + b_scr[0:1, :]
    o_ref[0] = res.astype(o_ref.dtype)


@jax.jit
def pallas_gated_mix__sliding_block_cached__dense_activation_gelu__decode_kernel(
    A_x: jax.Array,
    A_k_cache: jax.Array,
    A_v_cache: jax.Array,
    A_wq: jax.Array,
    A_wo: jax.Array,
    B_x: jax.Array,
    B_w1: jax.Array,
    B_b1: jax.Array,
    B_w2: jax.Array,
    B_b2: jax.Array,
    gate_w: jax.Array,
):
    del B_x
    cfg = DEFAULT
    bsz, sq, d_model = A_x.shape
    _, n_heads, sk, dh = A_k_cache.shape
    d_ff = B_w1.shape[1]
    win = min(4096, max(256, sk // 4))
    n_pairs = n_heads // 2
    pair = 2 * dh
    k_t = jnp.swapaxes(A_k_cache, 2, 3).reshape(n_pairs, pair, sk)
    v_t = jnp.swapaxes(A_v_cache, 2, 3).reshape(n_pairs, pair, sk)
    kernel = functools.partial(_kernel, n_pairs=n_pairs, dh=dh, win=win, sk=sk, cfg=cfg)
    any_spec = pl.BlockSpec(memory_space=pl.ANY)
    n_sem = cfg["L"] + 9 + 2 * (pair // cfg["R"]) // cfg["sgrp"]
    return pl.pallas_call(
        kernel,
        out_shape=jax.ShapeDtypeStruct((bsz, sq, d_model), A_x.dtype),
        in_specs=[any_spec] * 10,
        out_specs=pl.BlockSpec(memory_space=pltpu.VMEM),
        scratch_shapes=[
            pltpu.VMEM(A_x.shape, BF16),
            pltpu.VMEM(B_b1.shape, BF16),
            pltpu.VMEM(B_b2.shape, BF16),
            pltpu.VMEM(gate_w.shape, BF16),
            pltpu.VMEM((d_model, pair), BF16),
            pltpu.VMEM((d_model, pair), BF16),
            pltpu.VMEM((pair, d_model), BF16),
            pltpu.VMEM(B_w1.shape, BF16),
            pltpu.VMEM(B_w2.shape, BF16),
            pltpu.VMEM((pair, win), BF16),
            pltpu.VMEM((pair, win), BF16),
            pltpu.VMEM((8, d_model), BF16),
            pltpu.VMEM((pair, 128), F32),
            pltpu.VMEM((16, win), F32),
            pltpu.VMEM((pair, 128), F32),
            pltpu.VMEM((8, d_ff), BF16),
            pltpu.VMEM((8, d_model), F32),
            pltpu.SemaphoreType.DMA((n_sem,)),
        ],
        compiler_params=pltpu.CompilerParams(
            vmem_limit_bytes=64 * 1024 * 1024,
            disable_semaphore_checks=True,
            disable_bounds_checks=True),
    )(A_x, k_t, v_t, A_wq, A_wo, B_w1, B_b1, B_w2, B_b2, gate_w)
```

```python
import functools

import jax
import jax.numpy as jnp
from jax import lax
import jax.experimental.pallas as pl
import jax.experimental.pallas.tpu as pltpu

F32 = jnp.float32
BF16 = jnp.bfloat16

DEFAULT = dict(R=16, split=1792, strip=128, lead=6, sgrp=2, L=24, nw=8, compute=True,
               q_step=8, ffn_step=4, ffn_gap=12, fin=4, wq_stride=16, shift=8, pace=0, wq0_n=16,
               w2_last=True)


def _gelu_tanh(x):
    c = 0.7978845608028654
    return 0.5 * x * (1.0 + jnp.tanh(c * (x + 0.044715 * (x * x * x))))


def _spread(units, nsteps):
    out, done = [], 0
    for s in range(nsteps):
        upto = (units * (s + 1)) // nsteps
        out.append(range(done, upto))
        done = upto
    return out


def _tree_sum(terms):
    while len(terms) > 1:
        terms = [terms[u] + terms[u + 1] if u + 1 < len(terms) else terms[u]
                 for u in range(0, len(terms), 2)]
    return terms[0]


def _kernel(x_hbm, k_hbm, v_hbm, wq_hbm, wo_hbm, w1_hbm, b1_hbm, w2_hbm, b2_hbm,
            gw_hbm, o_ref,
            x_v, b1_v, b2_v, gw_v, wq_v, wo_v, w1_v, w2_v, kbuf, vbuf,
            x8_scr, qcol, s_scr, oacc, h_scr, b_scr, sems,
            *, n_pairs, dh, win, sk, cfg):
    R, L, nw, compute, fin = cfg["R"], cfg["L"], cfg["nw"], cfg["compute"], cfg["fin"]
    split, strip, lead, sgrp = cfg["split"], cfg["strip"], cfg["lead"], cfg["sgrp"]
    d_model = x_v.shape[-1]
    d_ff = w1_v.shape[1]
    pair = 2 * dh
    scale = float(dh) ** -0.5
    dma_parts = [(0, split), (split + strip, win - split - strip)]
    cmp_parts = [(0, split), (split, win - split)]
    ns = pair // R
    nh = ns // 2
    half = 2 * ns
    n_steps = 2 * half
    n_g = R // 8
    srows = pair // half
    n_qt, n_ot = d_model // 8, pair // 8
    wo_grp = fin * n_g
    w2_late = pair if cfg["w2_last"] else 0
    w2_early = d_ff - w2_late
    w1_per, w2_per = d_model // 8 // nw, w2_early // 8 // nw
    assert n_steps % L == 0 and (not strip or srows % 8 == 0) and half % sgrp == 0 and ns % fin == 0
    assert w1_per * nw * 8 == d_model and w2_per * nw * 8 == w2_early and nw < n_pairs - 1
    assert not strip or (0 < lead <= half // 2 and sgrp % (R // srows) == 0 and lead % sgrp == 0)
    steps = [(ph, t, j) for ph in range(2) for t in range(2) for j in range(ns)]
    S_WQ, S_W1, S_W2, S_X, S_SM = (L + t for t in range(5))
    S_ST = S_SM + 3
    S_WO = S_ST + half // sgrp
    bufs = ((k_hbm, kbuf), (v_hbm, vbuf))

    def kv(i, s):
        ph, t, j = steps[s]
        src, dst = bufs[ph]
        o, c = dma_parts[t]
        rows = pl.ds(j * R, R)
        return pltpu.make_async_copy(src.at[i, rows, pl.ds(sk - win + o, c)],
                                     dst.at[rows, pl.ds(o, c)], sems.at[s % L])

    def strip_copy(i, ph, u, n=1):
        src, dst = bufs[ph]
        rows = pl.ds(u * srows, n * srows)
        return pltpu.make_async_copy(src.at[i, rows, pl.ds(sk - win + split, strip)],
                                     dst.at[rows, pl.ds(split, strip)],
                                     sems.at[S_ST + u // sgrp])

    st = cfg["wq_stride"]
    wq_order = [b + k for b in range(st) for k in range(0, n_qt, st) if b + k < n_qt]
    assert sorted(wq_order) == list(range(n_qt))

    def wq_piece(i, u):
        rows = pl.ds(wq_order[u] * 8, 8)
        cols = pl.ds(i * pair if isinstance(i, int) else pl.multiple_of(i * pair, 128), pair)
        return pltpu.make_async_copy(wq_hbm.at[rows, cols], wq_v.at[rows], sems.at[S_WQ])

    def wo_piece(i, u, n=1):
        return pltpu.make_async_copy(
            wo_hbm.at[pl.ds(pl.multiple_of(i * pair + u * 8, 8), n * 8)],
            wo_v.at[pl.ds(u * 8, n * 8)], sems.at[S_WO + u // wo_grp])

    def w1_piece(i, u):
        rows = pl.ds(pl.multiple_of((i * w1_per + u // 2) * 8, 8), 8)
        cols = pl.ds((u % 2) * (d_ff // 2), d_ff // 2)
        return pltpu.make_async_copy(w1_hbm.at[rows, cols], w1_v.at[rows, cols], sems.at[S_W1])

    def w2_piece(i, u):
        rows = pl.ds(pl.multiple_of((i * w2_per + u) * 8, 8), 8)
        return pltpu.make_async_copy(w2_hbm.at[rows], w2_v.at[rows], sems.at[S_W2])

    def w2_rows(r0, n):
        rows = pl.ds(r0, n)
        return pltpu.make_async_copy(w2_hbm.at[rows], w2_v.at[rows], sems.at[S_W2])

    def wait_all(buf, sem):
        pltpu.make_async_copy(buf, buf, sems.at[sem]).wait()

    wq_sp = _spread(n_qt, half)
    wo_sp = _spread(n_ot, half)
    shift = cfg["shift"]
    assert 0 <= shift < half - cfg["q_step"]
    w2l_sp = _spread(w2_late // 8, half)
    w1_sp = _spread(2 * w1_per, half)
    w2_sp = _spread(w2_per, half)

    x_copy = pltpu.make_async_copy(x_hbm, x_v, sems.at[S_X])
    small = [pltpu.make_async_copy(gw_hbm, gw_v, sems.at[S_SM]),
             pltpu.make_async_copy(b1_hbm, b1_v, sems.at[S_SM + 1]),
             pltpu.make_async_copy(b2_hbm, b2_v, sems.at[S_SM + 2])]

    if cfg["pace"]:
        for s in range(L):
            kv(0, s).start(priority=1)
            if s == 1:
                x_copy.start()
                small[0].start()
        for grp in _spread(n_qt, cfg["wq0_n"]):
            for u in grp:
                wq_piece(0, u).start()
            pl.delay(cfg["pace"])
    else:
        x_copy.start()
        small[0].start()
        pltpu.make_async_copy(wq_hbm.at[:, pl.ds(0, pair)], wq_v, sems.at[S_WQ]).start()
        for s in range(L):
            kv(0, s).start(priority=1)
    for cp in small[1:]:
        cp.start()
    for u in range(0, lead if strip else 0, sgrp):
        strip_copy(0, 0, u, sgrp).start()

    def make_qcol():
        q8 = jnp.dot(x8_scr[...], wq_v[...], preferred_element_type=F32)
        q8 = q8.astype(BF16).astype(F32)
        qb = jnp.concatenate([q8] * 16, axis=0)
        qcol[...] = qb.T

    x_copy.wait()
    small[0].wait()
    x8_scr[...] = jnp.broadcast_to(x_v[0], (8, d_model))
    gate = jnp.sum(x8_scr[...].astype(F32) * gw_v[...].astype(F32).reshape(1, -1),
                   axis=-1, keepdims=True)
    gate = 1.0 / (1.0 + jnp.exp(-gate))
    wait_all(wq_v, S_WQ)
    if compute:
        make_qcol()
    for v in range(shift):
        for u in wq_sp[v]:
            wq_piece(1, u).start()
    for cp in small[1:]:
        cp.wait()

    def pair_body(i, out):
        more = i + 1 < n_pairs
        last = i + 1 == n_pairs
        m_vec = [None, None]
        m = [None, None]
        lsum = [None, None]
        inv_l = [None, None]
        s_acc = p = out_h = None
        pending = []

        def finalize(pend, out_h, out):
            accs, r0, hh, jj = pend
            wf = wo_v[r0:r0 + R, :].astype(F32)
            for g in range(n_g):
                term = wf[8 * g:8 * g + 8, :] * jnp.sum(accs[g], axis=-1, keepdims=True)
                out_h = term if (jj == 0 and g == 0) else out_h + term
            if jj == nh - 1:
                out = out + out_h * inv_l[hh]
            return out_h, out

        for s in range(n_steps):
            ph, t, j = steps[s]
            o, c = cmp_parts[t]
            n_cb = c // 128
            hh, jj = j // nh, j % nh
            r0 = j * R

            kv(i, s).wait()
            if s + L < n_steps:
                kv(i, s + L).start(priority=1)
            else:
                @pl.when(more)
                def _():
                    kv(i + 1, s + L - n_steps).start(priority=1)
            su = s + lead
            if not strip:
                pass
            elif su < n_steps:
                strip_copy(i, su // half, su % half).start()
            else:
                @pl.when(more)
                def _():
                    strip_copy(i + 1, 0, su - n_steps).start()
            v = (s + shift) % n_steps
            if v < half:
                ahead = 1 if s + shift < n_steps else 2

                @pl.when(i + ahead < n_pairs)
                def _():
                    for u in wq_sp[v]:
                        wq_piece(i + ahead, u).start()
                if w2_late:
                    @pl.when(i + ahead == n_pairs)
                    def _():
                        for u in w2l_sp[v]:
                            w2_rows(w2_early + u * 8, 8).start()
            else:
                for u in wo_sp[v - half]:
                    wo_piece(i, u).start()
            sp, fn = (w1_sp, w1_piece) if s % 2 == 0 else (w2_sp, w2_piece)
            if len(sp[s // 2]):
                @pl.when(i < nw)
                def _():
                    for u in sp[s // 2]:
                        fn(i, u).start()

            if s == half + cfg["q_step"]:
                @pl.when(more)
                def _():
                    wait_all(wq_v, S_WQ)
                    if compute:
                        make_qcol()
                if w2_late:
                    @pl.when(last)
                    def _():
                        w2_rows(w2_early, w2_late).wait()
                        if compute:
                            b = jnp.dot(h_scr[:, w2_early:], w2_v[w2_early:, :],
                                        preferred_element_type=F32)
                            b_scr[...] += b * (1.0 - gate)
            if s == cfg["ffn_step"]:
                @pl.when(i == nw)
                def _():
                    wait_all(w1_v, S_W1)
                    if compute:
                        h = jnp.dot(x8_scr[...], w1_v[...], preferred_element_type=F32)
                        h = h + b1_v[...].astype(F32).reshape(1, -1)
                        h_scr[...] = _gelu_tanh(h).astype(BF16)
            if s == cfg["ffn_step"] + cfg["ffn_gap"]:
                @pl.when(i == nw)
                def _():
                    w2_rows(0, w2_early).wait()
                    if compute:
                        b = jnp.dot(h_scr[:, :w2_early], w2_v[:w2_early, :],
                                    preferred_element_type=F32)
                        b = b + b2_v[...].astype(F32).reshape(1, -1)
                        b_scr[...] = b * (1.0 - gate)
            if strip and t == 1 and (r0 // srows) % sgrp == 0:
                strip_copy(i, ph, r0 // srows, sgrp).wait()
            do_fin = ph == 1 and t == 1 and ((j > 0 and j % fin == 0) or j == ns - 1)
            if do_fin:
                grp = (j - 1) // fin
                wo_piece(i, grp * wo_grp, wo_grp).wait()
            if not compute:
                continue
            if do_fin:
                for pend in pending:
                    out_h, out = finalize(pend, out_h, out)
                pending = []
            if ph == 0:
                kf = kbuf[r0:r0 + R, o:o + c].astype(F32)
                qc = qcol[r0:r0 + R, :]
                for g in range(n_g):
                    qg = qc[8 * g:8 * g + 8]
                    term = [kf[8 * g:8 * g + 8, cb * 128:(cb + 1) * 128] * qg for cb in range(n_cb)]
                    if jj == 0 and g == 0:
                        s_acc = term
                    else:
                        s_acc = [u + v for u, v in zip(s_acc, term)]
                if jj == nh - 1:
                    for cb in range(n_cb):
                        z = s_acc[cb]
                        z = z + pltpu.roll(z, 4, 0)
                        z = z + pltpu.roll(z, 2, 0)
                        z = z + pltpu.roll(z, 1, 0)
                        s_scr[hh * 8:(hh + 1) * 8, o + cb * 128:o + (cb + 1) * 128] = z
                        m_vec[hh] = z if m_vec[hh] is None else jnp.maximum(m_vec[hh], z)
                    if t == 1:
                        m[hh] = jnp.max(m_vec[hh], axis=-1, keepdims=True)
            else:
                if jj == 0:
                    sv = s_scr[hh * 8:(hh + 1) * 8, o:o + c]
                    pv = jnp.exp((sv - m[hh]) * scale)
                    p = [pv[:, cb * 128:(cb + 1) * 128] for cb in range(n_cb)]
                    ps = _tree_sum(list(p))
                    lsum[hh] = ps if lsum[hh] is None else lsum[hh] + ps
                    if t == 1:
                        inv_l[hh] = gate / jnp.sum(lsum[hh], axis=-1, keepdims=True)
                vf = vbuf[r0:r0 + R, o:o + c].astype(F32)
                accs = []
                for g in range(n_g):
                    terms = [vf[8 * g:8 * g + 8, cb * 128:(cb + 1) * 128] * p[cb] for cb in range(n_cb)]
                    if t > 0:
                        terms.append(oacc[r0 + 8 * g:r0 + 8 * g + 8, :])
                    accs.append(_tree_sum(terms))
                if t == 0:
                    for g in range(n_g):
                        oacc[r0 + 8 * g:r0 + 8 * g + 8, :] = accs[g]
                else:
                    pending.append((accs, r0, hh, jj))
                    if s == n_steps - 1:
                        out_h, out = finalize(pending.pop(), out_h, out)
        return out

    out = lax.fori_loop(0, n_pairs, pair_body, jnp.zeros((8, d_model), F32))

    res = jnp.sum(out, axis=0, keepdims=True)
    if compute:
        res = res + b_scr[0:1, :]
    o_ref[0] = res.astype(o_ref.dtype)


@jax.jit
def pallas_gated_mix__sliding_block_cached__dense_activation_gelu__decode_kernel(
    A_x: jax.Array,
    A_k_cache: jax.Array,
    A_v_cache: jax.Array,
    A_wq: jax.Array,
    A_wo: jax.Array,
    B_x: jax.Array,
    B_w1: jax.Array,
    B_b1: jax.Array,
    B_w2: jax.Array,
    B_b2: jax.Array,
    gate_w: jax.Array,
):
    del B_x
    cfg = DEFAULT
    bsz, sq, d_model = A_x.shape
    _, n_heads, sk, dh = A_k_cache.shape
    d_ff = B_w1.shape[1]
    win = min(4096, max(256, sk // 4))
    n_pairs = n_heads // 2
    pair = 2 * dh
    k_t = jnp.swapaxes(A_k_cache, 2, 3).reshape(n_pairs, pair, sk)
    v_t = jnp.swapaxes(A_v_cache, 2, 3).reshape(n_pairs, pair, sk)
    kernel = functools.partial(_kernel, n_pairs=n_pairs, dh=dh, win=win, sk=sk, cfg=cfg)
    any_spec = pl.BlockSpec(memory_space=pl.ANY)
    ns = pair // cfg["R"]
    n_sem = cfg["L"] + 7 + 2 * ns // cfg["sgrp"] + ns // cfg["fin"]
    return pl.pallas_call(
        kernel,
        out_shape=jax.ShapeDtypeStruct((bsz, sq, d_model), A_x.dtype),
        in_specs=[any_spec] * 10,
        out_specs=pl.BlockSpec(memory_space=pltpu.VMEM),
        scratch_shapes=[
            pltpu.VMEM(A_x.shape, BF16),
            pltpu.VMEM(B_b1.shape, BF16),
            pltpu.VMEM(B_b2.shape, BF16),
            pltpu.VMEM(gate_w.shape, BF16),
            pltpu.VMEM((d_model, pair), BF16),
            pltpu.VMEM((pair, d_model), BF16),
            pltpu.VMEM(B_w1.shape, BF16),
            pltpu.VMEM(B_w2.shape, BF16),
            pltpu.VMEM((pair, win), BF16),
            pltpu.VMEM((pair, win), BF16),
            pltpu.VMEM((8, d_model), BF16),
            pltpu.VMEM((pair, 128), F32),
            pltpu.VMEM((16, win), F32),
            pltpu.VMEM((pair, 128), F32),
            pltpu.VMEM((8, d_ff), BF16),
            pltpu.VMEM((8, d_model), F32),
            pltpu.SemaphoreType.DMA((n_sem,)),
        ],
        compiler_params=pltpu.CompilerParams(
            vmem_limit_bytes=64 * 1024 * 1024,
            disable_semaphore_checks=True,
            disable_bounds_checks=True),
    )(A_x, k_t, v_t, A_wq, A_wo, B_w1, B_b1, B_w2, B_b2, gate_w)
```

```python
import functools

import jax
import jax.numpy as jnp
from jax import lax
import jax.experimental.pallas as pl
import jax.experimental.pallas.tpu as pltpu

F32 = jnp.float32
BF16 = jnp.bfloat16

_R = 16
_SPLIT = 1792
_STRIP = 128
_LEAD = 8
_SGRP = 2
_LOOK = 24
_NW = 8
_SHIFT = 4
_Q_STEP = 8
_FFN_STEPS = (4, 16)
_FIN = 8
_TAIL = 4
_WQ_STRIDE = 16


def _gelu_tanh(x):
    c = 0.7978845608028654
    return 0.5 * x * (1.0 + jnp.tanh(c * (x + 0.044715 * (x * x * x))))


def _spread(units, nsteps):
    cuts = [(units * s) // nsteps for s in range(nsteps + 1)]
    return [range(cuts[s], cuts[s + 1]) for s in range(nsteps)]


def _fold_lanes(x, op):
    extra = []
    while x.shape[1] > 128:
        n = x.shape[1] // 128
        if n % 2:
            extra.append(x[:, (n - 1) * 128:])
            n -= 1
        x = op(x[:, :n * 64], x[:, n * 64:n * 128])
    for e in extra:
        x = op(x, e)
    return x


def _num_sems(pair):
    ns = pair // _R
    return _LOOK + 7 + 2 * ns // _SGRP + ns // _FIN + 1


def _kernel(x_hbm, k_hbm, v_hbm, wq_hbm, wo_hbm, w1_hbm, b1_hbm, w2_hbm, b2_hbm,
            gw_hbm, o_ref,
            x_v, b1_v, b2_v, gw_v, wq_v, wo_v, w1_v, w2_v, kbuf, vbuf,
            x8_scr, qcol, s_scr, oacc, h_scr, b_scr, sems,
            *, n_pairs, dh, win, sk):
    d_model = x_v.shape[-1]
    d_ff = w1_v.shape[1]
    pair = 2 * dh
    scale = float(dh) ** -0.5
    dma_parts = ((0, _SPLIT), (_SPLIT + _STRIP, win - _SPLIT - _STRIP))
    cmp_parts = ((0, _SPLIT), (_SPLIT, win - _SPLIT))
    ns = pair // _R
    nh = ns // 2
    half = 2 * ns
    n_steps = 2 * half
    n_g = _R // 8
    srows = pair // half
    n_qt, n_ot = d_model // 8, pair // 8
    wo_grp = _FIN * n_g
    w2_early = d_ff - pair
    w1_per, w2_per = d_model // 8 // _NW, w2_early // 8 // _NW
    assert dh % _R == 0 and n_steps % _LOOK == 0 and ns % _FIN == 0
    assert srows % 8 == 0 and half % _SGRP == 0 and _SGRP % (_R // srows) == 0
    assert _LEAD % _SGRP == 0 and _LEAD <= half // 2 and _SHIFT + _Q_STEP < half
    assert w1_per * _NW * 8 == d_model and w2_per * _NW * 8 == w2_early
    assert _NW < n_pairs - 1 and _TAIL % n_g == 0 and _TAIL < wo_grp
    steps = [(ph, t, j) for ph in range(2) for t in range(2) for j in range(ns)]
    s_wq, s_w1, s_w2, s_small = _LOOK, _LOOK + 1, _LOOK + 2, _LOOK + 3
    s_strip = s_small + 4
    s_wo = s_strip + half // _SGRP
    bufs = ((k_hbm, kbuf), (v_hbm, vbuf))

    def kv_copy(i, s):
        ph, t, j = steps[s]
        src, dst = bufs[ph]
        o, c = dma_parts[t]
        rows = pl.ds(j * _R, _R)
        return pltpu.make_async_copy(src.at[i, rows, pl.ds(sk - win + o, c)],
                                     dst.at[rows, pl.ds(o, c)], sems.at[s % _LOOK])

    def strip_copy(i, ph, u, n=1):
        src, dst = bufs[ph]
        rows = pl.ds(u * srows, n * srows)
        return pltpu.make_async_copy(src.at[i, rows, pl.ds(sk - win + _SPLIT, _STRIP)],
                                     dst.at[rows, pl.ds(_SPLIT, _STRIP)],
                                     sems.at[s_strip + u // _SGRP])

    wq_order = [u for b in range(_WQ_STRIDE) for u in range(b, n_qt, _WQ_STRIDE)]

    def wq_copy(i, u):
        rows = pl.ds(wq_order[u] * 8, 8)
        col0 = i * pair if isinstance(i, int) else pl.multiple_of(i * pair, 128)
        return pltpu.make_async_copy(wq_hbm.at[rows, pl.ds(col0, pair)],
                                     wq_v.at[rows], sems.at[s_wq])

    def wo_copy(i, u, n=1):
        grp = u // wo_grp + (1 if u >= n_ot - _TAIL else 0)
        return pltpu.make_async_copy(
            wo_hbm.at[pl.ds(pl.multiple_of(i * pair + u * 8, 8), n * 8)],
            wo_v.at[pl.ds(u * 8, n * 8)], sems.at[s_wo + grp])

    def w1_copy(i, u):
        rows = pl.ds(pl.multiple_of((i * w1_per + u // 2) * 8, 8), 8)
        cols = pl.ds((u % 2) * (d_ff // 2), d_ff // 2)
        return pltpu.make_async_copy(w1_hbm.at[rows, cols], w1_v.at[rows, cols],
                                     sems.at[s_w1])

    def w2_rows(r0, n):
        rows = pl.ds(r0, n)
        return pltpu.make_async_copy(w2_hbm.at[rows], w2_v.at[rows], sems.at[s_w2])

    def w2_copy(i, u):
        return w2_rows(pl.multiple_of((i * w2_per + u) * 8, 8), 8)

    def wait_all(buf, sem):
        pltpu.make_async_copy(buf, buf, sems.at[sem]).wait()

    wq_sp = _spread(n_qt, half)
    wo_sp = _spread(n_ot, half)
    w1_sp = _spread(2 * w1_per, half)
    w2_sp = _spread(w2_per, half)

    small = [pltpu.make_async_copy(src, dst, sems.at[s_small + u]) for u, (src, dst) in
             enumerate(((x_hbm, x_v), (gw_hbm, gw_v), (b1_hbm, b1_v), (b2_hbm, b2_v)))]

    small[0].start()
    small[1].start()
    pltpu.make_async_copy(wq_hbm.at[:, pl.ds(0, pair)], wq_v, sems.at[s_wq]).start()
    for s in range(_LOOK):
        kv_copy(0, s).start(priority=1)
    small[2].start()
    small[3].start()
    for u in range(0, _LEAD, _SGRP):
        strip_copy(0, 0, u, _SGRP).start()

    def make_qcol():
        q8 = jnp.dot(x8_scr[...], wq_v[...], preferred_element_type=F32)
        q8 = q8.astype(BF16).astype(F32)
        qcol[...] = jnp.concatenate([q8] * 16, axis=0).T

    small[0].wait()
    small[1].wait()
    x8_scr[...] = jnp.broadcast_to(x_v[0], (8, d_model))
    gate = jnp.sum(x8_scr[...].astype(F32) * gw_v[...].astype(F32).reshape(1, -1),
                   axis=-1, keepdims=True)
    gate = 1.0 / (1.0 + jnp.exp(-gate))
    wait_all(wq_v, s_wq)
    make_qcol()
    for v in range(_SHIFT):
        for u in wq_sp[v]:
            wq_copy(1, u).start()
    small[2].wait()
    small[3].wait()

    def pair_body(i, out):
        more = i + 1 < n_pairs
        last = i + 1 == n_pairs
        m_vec, m, lsum, coef = [None] * 2, [None] * 2, [None] * 2, [None] * 2
        s_acc = p = out_h = None
        pending = []

        def project(batch, out_h, out):
            for o_col, r0, hh, jj in batch:
                prod = wo_v[r0:r0 + _R, :].astype(F32) * o_col
                for g in range(n_g):
                    term = prod[8 * g:8 * g + 8]
                    out_h = term if (jj == 0 and g == 0) else out_h + term
                if jj == nh - 1:
                    out = out + out_h * coef[hh]
            return out_h, out

        def reduce_pending():
            return [(jnp.sum(a, axis=-1, keepdims=True), r0, hh, jj)
                    for a, r0, hh, jj in pending]

        for s in range(n_steps):
            ph, t, j = steps[s]
            o, c = cmp_parts[t]
            hh, jj = j // nh, j % nh
            r0 = j * _R
            flush = ph == 1 and t == 1 and j > 0 and j % _FIN == 0

            if t == 1 and (r0 // srows) % _SGRP == 0:
                strip_copy(i, ph, r0 // srows, _SGRP).wait()
            if flush:
                wo_copy(i, (j // _FIN - 1) * wo_grp, wo_grp).wait()
            kv_copy(i, s).wait()
            if s + _LOOK < n_steps:
                kv_copy(i, s + _LOOK).start(priority=1)
            else:
                @pl.when(more)
                def _():
                    kv_copy(i + 1, s + _LOOK - n_steps).start(priority=1)
            su = s + _LEAD
            if su < n_steps:
                strip_copy(i, su // half, su % half).start()
            else:
                @pl.when(more)
                def _():
                    strip_copy(i + 1, 0, su - n_steps).start()
            v = (s + _SHIFT) % n_steps
            if v < half:
                nxt = i + (1 if s + _SHIFT < n_steps else 2)

                @pl.when(nxt < n_pairs)
                def _():
                    for u in wq_sp[v]:
                        wq_copy(nxt, u).start()

                @pl.when(nxt == n_pairs)
                def _():
                    for u in wo_sp[v]:
                        w2_rows(w2_early + u * 8, 8).start()
            else:
                for u in wo_sp[v - half]:
                    if u < n_ot - wo_grp:
                        wo_copy(i, u).start()
                    else:
                        @pl.when(more)
                        def _():
                            wo_copy(i, u).start()
            if s + _LOOK == n_steps - 1:
                @pl.when(last)
                def _():
                    wo_copy(i, n_ot - wo_grp, wo_grp - _TAIL).start(priority=1)
                    wo_copy(i, n_ot - _TAIL, _TAIL).start(priority=1)
            sp, copy = (w1_sp, w1_copy) if s % 2 == 0 else (w2_sp, w2_copy)
            if len(sp[s // 2]):
                @pl.when(i < _NW)
                def _():
                    for u in sp[s // 2]:
                        copy(i, u).start()

            if s == half + _Q_STEP:
                @pl.when(more)
                def _():
                    wait_all(wq_v, s_wq)
                    make_qcol()

                @pl.when(last)
                def _():
                    w2_rows(w2_early, pair).wait()
                    b = jnp.dot(h_scr[:, w2_early:], w2_v[w2_early:, :],
                                preferred_element_type=F32)
                    b_scr[...] += b * (1.0 - gate)
            if s == _FFN_STEPS[0]:
                @pl.when(i == _NW)
                def _():
                    wait_all(w1_v, s_w1)
                    h = jnp.dot(x8_scr[...], w1_v[...], preferred_element_type=F32)
                    h = h + b1_v[...].astype(F32).reshape(1, -1)
                    h_scr[...] = _gelu_tanh(h).astype(BF16)
            if s == _FFN_STEPS[1]:
                @pl.when(i == _NW)
                def _():
                    w2_rows(0, w2_early).wait()
                    b = jnp.dot(h_scr[:, :w2_early], w2_v[:w2_early, :],
                                preferred_element_type=F32)
                    b = b + b2_v[...].astype(F32).reshape(1, -1)
                    b_scr[...] = b * (1.0 - gate)

            if flush:
                out_h, out = project(reduce_pending(), out_h, out)
                pending = []
            if ph == 0:
                prod = kbuf[r0:r0 + _R, o:o + c].astype(F32) * jnp.concatenate(
                    [qcol[r0:r0 + _R, :]] * (c // 128), axis=1)
                for g in range(n_g):
                    term = prod[8 * g:8 * g + 8]
                    s_acc = term if (jj == 0 and g == 0) else s_acc + term
                if jj == nh - 1:
                    for sh in (4, 2, 1):
                        s_acc = s_acc + pltpu.roll(s_acc, sh, 0)
                    s_scr[hh * 8:(hh + 1) * 8, o:o + c] = s_acc
                    z = _fold_lanes(s_acc, jnp.maximum)
                    m_vec[hh] = z if t == 0 else jnp.maximum(m_vec[hh], z)
                    if t == 1:
                        m[hh] = jnp.max(m_vec[hh], axis=-1, keepdims=True)
            else:
                if jj == 0:
                    p = jnp.exp((s_scr[hh * 8:(hh + 1) * 8, o:o + c] - m[hh]) * scale)
                    ps = _fold_lanes(p, jnp.add)
                    lsum[hh] = ps if t == 0 else lsum[hh] + ps
                    if t == 1:
                        coef[hh] = gate / jnp.sum(lsum[hh], axis=-1, keepdims=True)
                    p = jnp.concatenate([p] * n_g, axis=0)
                acc = _fold_lanes(vbuf[r0:r0 + _R, o:o + c].astype(F32) * p, jnp.add)
                if t == 0:
                    oacc[r0:r0 + _R, :] = acc
                else:
                    pending.append((acc + oacc[r0:r0 + _R, :], r0, hh, jj))

        batch = reduce_pending()
        n_first = len(batch) - _TAIL // n_g
        wo_copy(i, n_ot - wo_grp, wo_grp - _TAIL).wait()
        out_h, out = project(batch[:n_first], out_h, out)
        wo_copy(i, n_ot - _TAIL, _TAIL).wait()
        _, out = project(batch[n_first:], out_h, out)
        return out

    out = lax.fori_loop(0, n_pairs, pair_body, jnp.zeros((8, d_model), F32))

    res = jnp.sum(out, axis=0, keepdims=True) + b_scr[0:1, :]
    o_ref[0] = res.astype(o_ref.dtype)


@jax.jit
def pallas_gated_mix__sliding_block_cached__dense_activation_gelu__decode_kernel(
    A_x: jax.Array,
    A_k_cache: jax.Array,
    A_v_cache: jax.Array,
    A_wq: jax.Array,
    A_wo: jax.Array,
    B_x: jax.Array,
    B_w1: jax.Array,
    B_b1: jax.Array,
    B_w2: jax.Array,
    B_b2: jax.Array,
    gate_w: jax.Array,
):
    del B_x
    bsz, sq, d_model = A_x.shape
    _, n_heads, sk, dh = A_k_cache.shape
    d_ff = B_w1.shape[1]
    assert bsz == 1 and sq == 1 and n_heads % 2 == 0
    assert A_wq.shape == (d_model, n_heads * dh)
    win = min(4096, max(256, sk // 4))
    n_pairs = n_heads // 2
    pair = 2 * dh

    k_t = jnp.swapaxes(A_k_cache, 2, 3).reshape(n_pairs, pair, sk)
    v_t = jnp.swapaxes(A_v_cache, 2, 3).reshape(n_pairs, pair, sk)

    kernel = functools.partial(_kernel, n_pairs=n_pairs, dh=dh, win=win, sk=sk)
    return pl.pallas_call(
        kernel,
        out_shape=jax.ShapeDtypeStruct((bsz, sq, d_model), A_x.dtype),
        in_specs=[pl.BlockSpec(memory_space=pl.ANY)] * 10,
        out_specs=pl.BlockSpec(memory_space=pltpu.VMEM),
        scratch_shapes=[
            pltpu.VMEM(A_x.shape, BF16),
            pltpu.VMEM(B_b1.shape, BF16),
            pltpu.VMEM(B_b2.shape, BF16),
            pltpu.VMEM(gate_w.shape, BF16),
            pltpu.VMEM((d_model, pair), BF16),
            pltpu.VMEM((pair, d_model), BF16),
            pltpu.VMEM(B_w1.shape, BF16),
            pltpu.VMEM(B_w2.shape, BF16),
            pltpu.VMEM((pair, win), BF16),
            pltpu.VMEM((pair, win), BF16),
            pltpu.VMEM((8, d_model), BF16),
            pltpu.VMEM((pair, 128), F32),
            pltpu.VMEM((16, win), F32),
            pltpu.VMEM((pair, 128), F32),
            pltpu.VMEM((8, d_ff), BF16),
            pltpu.VMEM((8, d_model), F32),
            pltpu.SemaphoreType.DMA((_num_sems(pair),)),
        ],
        compiler_params=pltpu.CompilerParams(
            vmem_limit_bytes=48 * 1024 * 1024,
            disable_semaphore_checks=True,
            disable_bounds_checks=True),
    )(A_x, k_t, v_t, A_wq, A_wo, B_w1, B_b1, B_w2, B_b2, gate_w)
```

```python
import functools

import jax
import jax.numpy as jnp
from jax import lax
import jax.experimental.pallas as pl
import jax.experimental.pallas.tpu as pltpu

F32 = jnp.float32
BF16 = jnp.bfloat16

_R = 16
_SPLIT = 1792
_STRIP = 128
_LEAD = 8
_SGRP = 2
_LOOK = 24
_NW = 8
_SHIFT = 4
_Q_STEP = 8
_FFN_STEPS = (4, 16)
_FIN = 8
_TAIL = 4
_WQ_STRIDE = 16


def _gelu_tanh(x):
    c = 0.7978845608028654
    return 0.5 * x * (1.0 + jnp.tanh(c * (x + 0.044715 * (x * x * x))))


def _spread(units, nsteps):
    cuts = [(units * s) // nsteps for s in range(nsteps + 1)]
    return [range(cuts[s], cuts[s + 1]) for s in range(nsteps)]


def _fold_lanes(x, op):
    extra = []
    while x.shape[1] > 128:
        n = x.shape[1] // 128
        if n % 2:
            extra.append(x[:, (n - 1) * 128:])
            n -= 1
        x = op(x[:, :n * 64], x[:, n * 64:n * 128])
    for e in extra:
        x = op(x, e)
    return x


def _num_sems(pair):
    ns = pair // _R
    return _LOOK + 7 + 2 * ns // _SGRP + ns // _FIN + 1


def _compiler_params():
    base = dict(vmem_limit_bytes=48 * 1024 * 1024, disable_bounds_checks=True)
    try:
        return pltpu.CompilerParams(disable_semaphore_checks=True, **base)
    except TypeError:
        return pltpu.CompilerParams(**base)


def _kernel(x_hbm, k_hbm, v_hbm, wq_hbm, wo_hbm, w1_hbm, b1_hbm, w2_hbm, b2_hbm,
            gw_hbm, o_ref,
            x_v, b1_v, b2_v, gw_v, wq_v, wo_v, w1_v, w2_v, kbuf, vbuf,
            x8_scr, qcol, s_scr, oacc, h_scr, b_scr, sems,
            *, n_pairs, dh, win, sk):
    d_model = x_v.shape[-1]
    d_ff = w1_v.shape[1]
    pair = 2 * dh
    scale = float(dh) ** -0.5
    dma_parts = ((0, _SPLIT), (_SPLIT + _STRIP, win - _SPLIT - _STRIP))
    cmp_parts = ((0, _SPLIT), (_SPLIT, win - _SPLIT))
    ns = pair // _R
    nh = ns // 2
    half = 2 * ns
    n_steps = 2 * half
    n_g = _R // 8
    srows = pair // half
    n_qt, n_ot = d_model // 8, pair // 8
    wo_grp = _FIN * n_g
    w2_early = d_ff - pair
    w1_per, w2_per = d_model // 8 // _NW, w2_early // 8 // _NW
    assert dh % _R == 0 and n_steps % _LOOK == 0 and ns % _FIN == 0
    assert srows % 8 == 0 and half % _SGRP == 0 and _SGRP % (_R // srows) == 0
    assert _LEAD % _SGRP == 0 and _LEAD <= half // 2 and _SHIFT + _Q_STEP < half
    assert w1_per * _NW * 8 == d_model and w2_per * _NW * 8 == w2_early
    assert _NW < n_pairs - 1 and _TAIL % n_g == 0 and _TAIL < wo_grp
    steps = [(ph, t, j) for ph in range(2) for t in range(2) for j in range(ns)]
    s_wq, s_w1, s_w2, s_small = _LOOK, _LOOK + 1, _LOOK + 2, _LOOK + 3
    s_strip = s_small + 4
    s_wo = s_strip + half // _SGRP
    bufs = ((k_hbm, kbuf), (v_hbm, vbuf))

    def kv_copy(i, s):
        ph, t, j = steps[s]
        src, dst = bufs[ph]
        o, c = dma_parts[t]
        rows = pl.ds(j * _R, _R)
        return pltpu.make_async_copy(src.at[i, rows, pl.ds(sk - win + o, c)],
                                     dst.at[rows, pl.ds(o, c)], sems.at[s % _LOOK])

    def strip_copy(i, ph, u, n=1):
        src, dst = bufs[ph]
        rows = pl.ds(u * srows, n * srows)
        return pltpu.make_async_copy(src.at[i, rows, pl.ds(sk - win + _SPLIT, _STRIP)],
                                     dst.at[rows, pl.ds(_SPLIT, _STRIP)],
                                     sems.at[s_strip + u // _SGRP])

    wq_order = [u for b in range(_WQ_STRIDE) for u in range(b, n_qt, _WQ_STRIDE)]

    def wq_copy(i, u):
        rows = pl.ds(wq_order[u] * 8, 8)
        col0 = i * pair if isinstance(i, int) else pl.multiple_of(i * pair, 128)
        return pltpu.make_async_copy(wq_hbm.at[rows, pl.ds(col0, pair)],
                                     wq_v.at[rows], sems.at[s_wq])

    def wo_copy(i, u, n=1):
        grp = u // wo_grp + (1 if u >= n_ot - _TAIL else 0)
        return pltpu.make_async_copy(
            wo_hbm.at[pl.ds(pl.multiple_of(i * pair + u * 8, 8), n * 8)],
            wo_v.at[pl.ds(u * 8, n * 8)], sems.at[s_wo + grp])

    def w1_copy(i, u):
        rows = pl.ds(pl.multiple_of((i * w1_per + u // 2) * 8, 8), 8)
        cols = pl.ds((u % 2) * (d_ff // 2), d_ff // 2)
        return pltpu.make_async_copy(w1_hbm.at[rows, cols], w1_v.at[rows, cols],
                                     sems.at[s_w1])

    def w2_rows(r0, n):
        rows = pl.ds(r0, n)
        return pltpu.make_async_copy(w2_hbm.at[rows], w2_v.at[rows], sems.at[s_w2])

    def w2_copy(i, u):
        return w2_rows(pl.multiple_of((i * w2_per + u) * 8, 8), 8)

    def wait_all(buf, sem):
        pltpu.make_async_copy(buf, buf, sems.at[sem]).wait()

    wq_sp = _spread(n_qt, half)
    wo_sp = _spread(n_ot, half)
    w1_sp = _spread(2 * w1_per, half)
    w2_sp = _spread(w2_per, half)

    small = [pltpu.make_async_copy(src, dst, sems.at[s_small + u]) for u, (src, dst) in
             enumerate(((x_hbm, x_v), (gw_hbm, gw_v), (b1_hbm, b1_v), (b2_hbm, b2_v)))]

    small[0].start()
    small[1].start()
    pltpu.make_async_copy(wq_hbm.at[:, pl.ds(0, pair)], wq_v, sems.at[s_wq]).start()
    for s in range(_LOOK):
        kv_copy(0, s).start(priority=1)
    small[2].start()
    small[3].start()
    for u in range(0, _LEAD, _SGRP):
        strip_copy(0, 0, u, _SGRP).start()

    def make_qcol():
        q8 = jnp.dot(x8_scr[...], wq_v[...], preferred_element_type=F32)
        q8 = q8.astype(BF16).astype(F32)
        qcol[...] = jnp.concatenate([q8] * 16, axis=0).T

    small[0].wait()
    small[1].wait()
    x8_scr[...] = jnp.broadcast_to(x_v[0], (8, d_model))
    gate = jnp.sum(x8_scr[...].astype(F32) * gw_v[...].astype(F32).reshape(1, -1),
                   axis=-1, keepdims=True)
    gate = 1.0 / (1.0 + jnp.exp(-gate))
    wait_all(wq_v, s_wq)
    make_qcol()
    for v in range(_SHIFT):
        for u in wq_sp[v]:
            wq_copy(1, u).start()
    small[2].wait()
    small[3].wait()

    def pair_body(i, out):
        more = i + 1 < n_pairs
        last = i + 1 == n_pairs
        m_vec, m, lsum, coef = [None] * 2, [None] * 2, [None] * 2, [None] * 2
        s_acc = p = out_h = None
        pending = []

        def project(batch, out_h, out):
            for o_col, r0, hh, jj in batch:
                prod = wo_v[r0:r0 + _R, :].astype(F32) * o_col
                for g in range(n_g):
                    term = prod[8 * g:8 * g + 8]
                    out_h = term if (jj == 0 and g == 0) else out_h + term
                if jj == nh - 1:
                    out = out + out_h * coef[hh]
            return out_h, out

        def reduce_pending():
            return [(jnp.sum(a, axis=-1, keepdims=True), r0, hh, jj)
                    for a, r0, hh, jj in pending]

        for s in range(n_steps):
            ph, t, j = steps[s]
            o, c = cmp_parts[t]
            hh, jj = j // nh, j % nh
            r0 = j * _R
            flush = ph == 1 and t == 1 and j > 0 and j % _FIN == 0

            if t == 1 and (r0 // srows) % _SGRP == 0:
                strip_copy(i, ph, r0 // srows, _SGRP).wait()
            if flush:
                wo_copy(i, (j // _FIN - 1) * wo_grp, wo_grp).wait()
            kv_copy(i, s).wait()
            if s + _LOOK < n_steps:
                kv_copy(i, s + _LOOK).start(priority=1)
            else:
                @pl.when(more)
                def _():
                    kv_copy(i + 1, s + _LOOK - n_steps).start(priority=1)
            su = s + _LEAD
            if su < n_steps:
                strip_copy(i, su // half, su % half).start()
            else:
                @pl.when(more)
                def _():
                    strip_copy(i + 1, 0, su - n_steps).start()
            v = (s + _SHIFT) % n_steps
            if v < half:
                nxt = i + (1 if s + _SHIFT < n_steps else 2)

                @pl.when(nxt < n_pairs)
                def _():
                    for u in wq_sp[v]:
                        wq_copy(nxt, u).start()

                @pl.when(nxt == n_pairs)
                def _():
                    for u in wo_sp[v]:
                        w2_rows(w2_early + u * 8, 8).start()
            else:
                for u in wo_sp[v - half]:
                    if u < n_ot - wo_grp:
                        wo_copy(i, u).start()
                    else:
                        @pl.when(more)
                        def _():
                            wo_copy(i, u).start()
            if s + _LOOK == n_steps - 1:
                @pl.when(last)
                def _():
                    wo_copy(i, n_ot - wo_grp, wo_grp - _TAIL).start(priority=1)
                    wo_copy(i, n_ot - _TAIL, _TAIL).start(priority=1)
            sp, copy = (w1_sp, w1_copy) if s % 2 == 0 else (w2_sp, w2_copy)
            if len(sp[s // 2]):
                @pl.when(i < _NW)
                def _():
                    for u in sp[s // 2]:
                        copy(i, u).start()

            if s == half + _Q_STEP:
                @pl.when(more)
                def _():
                    wait_all(wq_v, s_wq)
                    make_qcol()

                @pl.when(last)
                def _():
                    w2_rows(w2_early, pair).wait()
                    b = jnp.dot(h_scr[:, w2_early:], w2_v[w2_early:, :],
                                preferred_element_type=F32)
                    b_scr[...] += b * (1.0 - gate)
            if s == _FFN_STEPS[0]:
                @pl.when(i == _NW)
                def _():
                    wait_all(w1_v, s_w1)
                    h = jnp.dot(x8_scr[...], w1_v[...], preferred_element_type=F32)
                    h = h + b1_v[...].astype(F32).reshape(1, -1)
                    h_scr[...] = _gelu_tanh(h).astype(BF16)
            if s == _FFN_STEPS[1]:
                @pl.when(i == _NW)
                def _():
                    w2_rows(0, w2_early).wait()
                    b = jnp.dot(h_scr[:, :w2_early], w2_v[:w2_early, :],
                                preferred_element_type=F32)
                    b = b + b2_v[...].astype(F32).reshape(1, -1)
                    b_scr[...] = b * (1.0 - gate)

            if flush:
                out_h, out = project(reduce_pending(), out_h, out)
                pending = []
            if ph == 0:
                prod = kbuf[r0:r0 + _R, o:o + c].astype(F32) * jnp.concatenate(
                    [qcol[r0:r0 + _R, :]] * (c // 128), axis=1)
                for g in range(n_g):
                    term = prod[8 * g:8 * g + 8]
                    s_acc = term if (jj == 0 and g == 0) else s_acc + term
                if jj == nh - 1:
                    for sh in (4, 2, 1):
                        s_acc = s_acc + pltpu.roll(s_acc, sh, 0)
                    s_scr[hh * 8:(hh + 1) * 8, o:o + c] = s_acc
                    z = _fold_lanes(s_acc, jnp.maximum)
                    m_vec[hh] = z if t == 0 else jnp.maximum(m_vec[hh], z)
                    if t == 1:
                        m[hh] = jnp.max(m_vec[hh], axis=-1, keepdims=True)
            else:
                if jj == 0:
                    p = jnp.exp((s_scr[hh * 8:(hh + 1) * 8, o:o + c] - m[hh]) * scale)
                    ps = _fold_lanes(p, jnp.add)
                    lsum[hh] = ps if t == 0 else lsum[hh] + ps
                    if t == 1:
                        coef[hh] = gate / jnp.sum(lsum[hh], axis=-1, keepdims=True)
                    p = jnp.concatenate([p] * n_g, axis=0)
                acc = _fold_lanes(vbuf[r0:r0 + _R, o:o + c].astype(F32) * p, jnp.add)
                if t == 0:
                    oacc[r0:r0 + _R, :] = acc
                else:
                    pending.append((acc + oacc[r0:r0 + _R, :], r0, hh, jj))

        batch = reduce_pending()
        n_first = len(batch) - _TAIL // n_g
        wo_copy(i, n_ot - wo_grp, wo_grp - _TAIL).wait()
        out_h, out = project(batch[:n_first], out_h, out)
        wo_copy(i, n_ot - _TAIL, _TAIL).wait()
        _, out = project(batch[n_first:], out_h, out)
        return out

    out = lax.fori_loop(0, n_pairs, pair_body, jnp.zeros((8, d_model), F32))

    res = jnp.sum(out, axis=0, keepdims=True) + b_scr[0:1, :]
    o_ref[0] = res.astype(o_ref.dtype)


@jax.jit
def pallas_gated_mix__sliding_block_cached__dense_activation_gelu__decode_kernel(
    A_x: jax.Array,
    A_k_cache: jax.Array,
    A_v_cache: jax.Array,
    A_wq: jax.Array,
    A_wo: jax.Array,
    B_x: jax.Array,
    B_w1: jax.Array,
    B_b1: jax.Array,
    B_w2: jax.Array,
    B_b2: jax.Array,
    gate_w: jax.Array,
):
    del B_x
    bsz, sq, d_model = A_x.shape
    _, n_heads, sk, dh = A_k_cache.shape
    d_ff = B_w1.shape[1]
    assert bsz == 1 and sq == 1 and n_heads % 2 == 0
    assert A_wq.shape == (d_model, n_heads * dh)
    win = min(4096, max(256, sk // 4))
    n_pairs = n_heads // 2
    pair = 2 * dh

    k_t = jnp.swapaxes(A_k_cache, 2, 3).reshape(n_pairs, pair, sk)
    v_t = jnp.swapaxes(A_v_cache, 2, 3).reshape(n_pairs, pair, sk)

    kernel = functools.partial(_kernel, n_pairs=n_pairs, dh=dh, win=win, sk=sk)
    return pl.pallas_call(
        kernel,
        out_shape=jax.ShapeDtypeStruct((bsz, sq, d_model), A_x.dtype),
        in_specs=[pl.BlockSpec(memory_space=pl.ANY)] * 10,
        out_specs=pl.BlockSpec(memory_space=pltpu.VMEM),
        scratch_shapes=[
            pltpu.VMEM(A_x.shape, BF16),
            pltpu.VMEM(B_b1.shape, BF16),
            pltpu.VMEM(B_b2.shape, BF16),
            pltpu.VMEM(gate_w.shape, BF16),
            pltpu.VMEM((d_model, pair), BF16),
            pltpu.VMEM((pair, d_model), BF16),
            pltpu.VMEM(B_w1.shape, BF16),
            pltpu.VMEM(B_w2.shape, BF16),
            pltpu.VMEM((pair, win), BF16),
            pltpu.VMEM((pair, win), BF16),
            pltpu.VMEM((8, d_model), BF16),
            pltpu.VMEM((pair, 128), F32),
            pltpu.VMEM((16, win), F32),
            pltpu.VMEM((pair, 128), F32),
            pltpu.VMEM((8, d_ff), BF16),
            pltpu.VMEM((8, d_model), F32),
            pltpu.SemaphoreType.DMA((_num_sems(pair),)),
        ],
        compiler_params=_compiler_params(),
    )(A_x, k_t, v_t, A_wq, A_wo, B_w1, B_b1, B_w2, B_b2, gate_w)
```
